```python
import os as _os
_os.environ.setdefault("JAX_PLATFORMS", "cpu")
import jax
import jax.numpy as jnp

def _softmax(x, axis=-1):
    return jax.nn.softmax(x, axis=axis)
def _gelu(x):
    return jax.nn.gelu(x, approximate=True)
def _silu(x):
    return jax.nn.silu(x)
def _sigmoid(x):
    return jax.nn.sigmoid(x)
def _layernorm(x, axis=-1, eps=1e-5):
    m = jnp.mean(x, axis=axis, keepdims=True)
    v = jnp.var(x, axis=axis, keepdims=True)
    return (x - m) / jnp.sqrt(v + eps)
def _scatter_add(tgt, idx, src, axis=0):
    return tgt.at[idx].add(src)
def _segment_sum(src, seg, n):
    return jax.ops.segment_sum(src, seg, n)
class _Rng:
    def __init__(self, key):
        self._k = key
    def _next(self):
        self._k, sub = jax.random.split(self._k)
        return sub
    def normal(self, shape):
        return jax.random.normal(self._next(), shape, dtype=jnp.bfloat16)
    def randint(self, lo, hi, shape):
        return jax.random.randint(self._next(), shape, lo, hi, dtype=jnp.int32)
    def uniform(self, shape, lo=0.0, hi=1.0):
        return jax.random.uniform(self._next(), shape, jnp.bfloat16, lo, hi)
    def permutation(self, n):
        return jax.random.permutation(self._next(), n)


kernel_name = 'standalone__groupnorm__sampling'

def setup_inputs():
    _rng = _Rng(jax.random.key(int.from_bytes(__import__("os").urandom(4), "little")))
    _w = (lambda a: (lambda t: t.astype(jnp.bfloat16) if jnp.issubdtype(t.dtype, jnp.floating) else t)(jnp.asarray(a)))
    B = 32
    G = 32
    cpg = max(1, 576 // G)
    C = G * cpg
    H, W = 32, 16
    return {
        "x": _w((lambda *s: _rng.normal(s) * 0.05)(B, C, H, W)),
        "g": _w((lambda *s: _rng.normal(s) * 0.05)(C) + 1.0),
        "b": _w((lambda *s: _rng.normal(s) * 0.05)(C)),
    }

def reference(x, g, b):
    G = 32
    B, C, H, W = x.shape[0], x.shape[1], x.shape[2], x.shape[3]
    xr = x.reshape(B, G, C // G, H, W)
    mu = xr.mean(axis=(2, 3, 4), keepdims=True)
    var = ((xr - mu) ** 2).mean(axis=(2, 3, 4), keepdims=True)
    xn = (xr - mu) / jnp.sqrt(var + 1e-5)
    xn = xn.reshape(B, C, H, W)
    return xn * g[None, :, None, None] + b[None, :, None, None]
```

```python
import functools
import jax
import jax.numpy as jnp
from jax import lax
from jax.experimental import pallas as pl
from jax.experimental.pallas import tpu as pltpu

G = 32
EPS = 1e-5

def make(L=24, OV=8, PR=8, PW=8, WFIRST=64, compute=True, wq=1):
    NS, NR = 8, 4
    def kernel(x_hbm, g_hbm, b_hbm, o_hbm, xbuf, obuf, gbuf, bbuf, mbuf, stat, scale, shift, sems):
        _, _, P, C = x_hbm.shape
        cpg = C // G
        inv_n = 1.0 / (cpg * P)
        NPR = P // PR
        NPW = P // PW
        TOT = NR * NPR

        def read_step(t, sem):
            r, j = t // NPR, t % NPR
            rows = pl.ds(pl.multiple_of(j * PR, PR), PR)
            for p in range(2):
                idx = (pl.ds(p * (NS // 2), NS // 2), r, rows)
                pltpu.make_async_copy(x_hbm.at[idx], xbuf.at[idx], sems.at[sem]).start(priority=p)

        def sem_of(t):
            return jnp.where(t >= TOT - OV, NR, t // NPR)

        def read_range(t0, n):
            def body(i, _):
                t = t0 + i
                read_step(t, sem_of(t))
            lax.fori_loop(0, n, body, None)

        def read_some(t0, n):
            for i in range(n):
                t = t0 + i
                @pl.when(t < TOT)
                def _():
                    read_step(t, sem_of(t))

        def write_range(t0, t1):
            def body(t, _):
                r, j = t // NPW, t % NPW
                rows = pl.ds(pl.multiple_of(j * PW, PW), PW)
                if wq == 1:
                    idx = (slice(None), r, rows)
                    pltpu.make_async_copy(obuf.at[idx], o_hbm.at[idx], sems.at[NR + 1]).start()
                else:
                    for p in range(2):
                        idx = (pl.ds(p * (NS // 2), NS // 2), r, rows)
                        pltpu.make_async_copy(obuf.at[idx], o_hbm.at[idx], sems.at[NR + 1]).start(priority=p)
            lax.fori_loop(t0, t1, body, None)

        def wait_rows(r, r0, n, sem):
            v = xbuf.at[:, r, pl.ds(r0, n)]
            pltpu.make_async_copy(v, v, sems.at[sem]).wait()

        read_range(0, 16)
        cg = pltpu.make_async_copy(g_hbm, gbuf, sems.at[NR + 2]); cg.start()
        cb = pltpu.make_async_copy(b_hbm, bbuf, sems.at[NR + 2]); cb.start()
        ri = lax.broadcasted_iota(jnp.int32, (C, C), 0).astype(jnp.float32)
        ci = lax.broadcasted_iota(jnp.int32, (C, C), 1).astype(jnp.float32)
        gr = jnp.floor((ri + 0.5) * (1.0 / cpg)); gc = jnp.floor((ci + 0.5) * (1.0 / cpg))
        mbuf[...] = jnp.where(gr == gc, 1.0, 0.0).astype(jnp.bfloat16)
        read_range(16, NPR + L - 16)
        cg.wait(); cb.wait()

        def group_sum(s):
            hi = s.astype(jnp.bfloat16); r1 = s - hi.astype(jnp.float32)
            mid = r1.astype(jnp.bfloat16); r2 = r1 - mid.astype(jnp.float32)
            lhs = jnp.concatenate([hi.astype(jnp.float32), mid.astype(jnp.float32), r2, jnp.zeros_like(s)], axis=0).astype(jnp.bfloat16)
            o = jnp.dot(lhs, mbuf[...], preferred_element_type=jnp.float32)
            return o[0:NS] + (o[NS:2 * NS] + o[2 * NS:3 * NS])

        k1, k2 = (NPR // NS) // 4, (3 * (NPR // NS)) // 8
        k3 = NPR // NS - k1 - k2

        def compute_round(r):
            t0 = (r + 1) * NPR + L
            def pass1(k, _):
                read_some(t0 + k * k1, k1)
                acc = jnp.zeros((16, C), jnp.float32)
                for i in range(P // 16):
                    acc = acc + xbuf[k, r, pl.ds(16 * i, 16), :].astype(jnp.float32)
                stat[pl.ds(k, 1), :] = jnp.sum(acc[0:8] + acc[8:16], axis=0, keepdims=True)
            lax.fori_loop(0, NS, pass1, None)
            mu = group_sum(stat[...]) * inv_n
            shift[...] = mu
            def pass2(k, _):
                read_some(t0 + NS * k1 + k * k2, k2)
                m = jnp.broadcast_to(shift[pl.ds(k, 1), :], (16, C))
                acc = jnp.zeros((16, C), jnp.float32)
                for i in range(P // 16):
                    d = xbuf[k, r, pl.ds(16 * i, 16), :].astype(jnp.float32) - m
                    acc = acc + d * d
                stat[pl.ds(k, 1), :] = jnp.sum(acc[0:8] + acc[8:16], axis=0, keepdims=True)
            lax.fori_loop(0, NS, pass2, None)
            var = group_sum(stat[...]) * inv_n
            gv = gbuf[...].astype(jnp.float32).reshape(1, C)
            sc = gv / jnp.sqrt(var + EPS)
            scale[...] = sc
            bv = bbuf[...].astype(jnp.float32).reshape(1, C)
            def pass3(k, _):
                read_some(t0 + NS * (k1 + k2) + k * k3, k3)
                m = jnp.broadcast_to(shift[pl.ds(k, 1), :], (16, C))
                a = jnp.broadcast_to(scale[pl.ds(k, 1), :], (16, C))
                bb = jnp.broadcast_to(bv, (16, C))
                for i in range(P // 16):
                    d = xbuf[k, r, pl.ds(16 * i, 16), :].astype(jnp.float32) - m
                    obuf[k, r, pl.ds(16 * i, 16), :] = (d * a + bb).astype(obuf.dtype)
            lax.fori_loop(0, NS, pass3, None)

        def round_body(r, _):
            @pl.when(r < NR - 1)
            def _():
                wait_rows(r, 0, P, r)
            @pl.when(r == NR - 1)
            def _():
                wait_rows(r, 0, P - OV * PR, r)
                write_range(0, WFIRST)
                if OV: wait_rows(r, P - OV * PR, OV * PR, NR)
            if compute:
                compute_round(r)
            else:
                t0 = (r + 1) * NPR + L
                read_range(t0, jnp.clip(TOT - t0, 0, NPR))
        lax.fori_loop(0, NR, round_body, None)
        write_range(WFIRST, NR * NPW)
        pltpu.make_async_copy(obuf, obuf, sems.at[NR + 1]).wait()

    def f(x, g, b):
        B, C, H, W = x.shape
        P = H * W
        shp = (NS, NR, P, C)
        xt = jnp.transpose(x, (0, 2, 3, 1)).reshape(shp)
        hbm = pl.BlockSpec(memory_space=pltpu.MemorySpace.HBM)
        y = pl.pallas_call(
            kernel,
            in_specs=[hbm, hbm, hbm],
            out_specs=hbm,
            out_shape=jax.ShapeDtypeStruct(shp, x.dtype),
            scratch_shapes=[
                pltpu.VMEM(shp, x.dtype), pltpu.VMEM(shp, x.dtype),
                pltpu.VMEM((C,), g.dtype), pltpu.VMEM((C,), b.dtype),
                pltpu.VMEM((C, C), jnp.bfloat16),
                pltpu.VMEM((NS, C), jnp.float32), pltpu.VMEM((NS, C), jnp.float32), pltpu.VMEM((NS, C), jnp.float32),
                pltpu.SemaphoreType.DMA((NR + 3,)),
            ],
            compiler_params=pltpu.CompilerParams(
                vmem_limit_bytes=64 * 2**20, disable_bounds_checks=True, disable_semaphore_checks=True),
        )(xt, g, b)
        return jnp.transpose(y.reshape(B, H, W, C), (0, 3, 1, 2))
    return f


@jax.jit
def pallas_standalone__groupnorm__sampling_kernel(x, g, b):
    return make()(x, g, b)
```

```python
import jax
import jax.numpy as jnp
from jax import lax
from jax.experimental import pallas as pl
from jax.experimental.pallas import tpu as pltpu

GROUPS = 32
EPS = 1e-5

ROUNDS = 4
READ_QUEUES = 2
READ_ROWS = 8
WRITE_ROWS = 16
READ_AHEAD = 52
OVERLAP = 10

SUBLANES = 8
LANES = 128


def _groupnorm_kernel(
    x_hbm, g_hbm, b_hbm, o_hbm, x_buf, o_buf, g_buf, b_buf, mean_ref, scale_ref, sems
):
    streams, rounds, npos, chans = x_hbm.shape
    group = chans // GROUPS
    early = rounds // 2
    steps = npos // READ_ROWS
    total = rounds * steps
    burst = steps // (2 * streams)
    head = npos - OVERLAP * READ_ROWS
    sem_late, sem_tail, sem_out, sem_affine = range(early, early + 4)

    def read_burst(t):
        r, j = lax.div(t, steps), lax.rem(t, steps)
        width = streams // READ_QUEUES
        for i in range(burst):
            s = jnp.where(t + i < total - OVERLAP, jnp.minimum(r, sem_late), sem_tail)
            start = pl.multiple_of((j + i) * READ_ROWS, READ_ROWS)
            for q in range(READ_QUEUES):
                idx = (pl.ds(q * width, width), r, pl.ds(start, READ_ROWS))
                copy = pltpu.make_async_copy(x_hbm.at[idx], x_buf.at[idx], sems.at[s])
                copy.start(priority=q)

    def read_steps(t0, t1):
        pl.loop(t0 // burst, t1 // burst)(lambda u: read_burst(u * burst))

    def wait_read(r, rows, s):
        idx = (slice(None), r, rows)
        pltpu.make_async_copy(x_hbm.at[idx], x_buf.at[idx], sems.at[s]).wait()

    def write_rounds(r0, r1):
        per_round = npos // WRITE_ROWS

        @pl.loop(r0 * per_round, r1 * per_round)
        def _(t):
            start = pl.multiple_of(lax.rem(t, per_round) * WRITE_ROWS, WRITE_ROWS)
            idx = (slice(None), lax.div(t, per_round), pl.ds(start, WRITE_ROWS))
            pltpu.make_async_copy(o_buf.at[idx], o_hbm.at[idx], sems.at[sem_out]).start()

    def group_mean(col_sums):
        width = pl.cdiv(chans, LANES) * LANES
        v = jnp.concatenate(
            [col_sums, jnp.zeros((streams, width - chans), jnp.float32)], axis=1
        )
        lane = lax.broadcasted_iota(jnp.int32, v.shape, 1).astype(jnp.float32)
        pos = lane - group * jnp.floor((lane + 0.5) * (1.0 / group))
        upto = v
        after = jnp.where(pos < group - 1, pltpu.roll(v, width - 1, 1), 0.0)
        d = 1
        while d < group:
            upto += jnp.where(pos >= d, pltpu.roll(upto, d, 1), 0.0)
            after += jnp.where(pos < group - d, pltpu.roll(after, width - d, 1), 0.0)
            d *= 2
        return (upto + after)[:, :chans] * (1.0 / (group * npos))

    def normalize_round(r):
        tiles = [pl.ds(i, SUBLANES) for i in range(0, npos, SUBLANES)]

        def load(s, rows):
            return x_buf[s, r, rows, :].astype(jnp.float32)

        def sample_row(ref, s):
            return jnp.broadcast_to(ref[pl.ds(s, 1), :], (SUBLANES, chans))

        def keep_reading(slot):
            t = (r + 1) * steps + READ_AHEAD + slot * burst
            pl.when(r < early)(lambda: read_burst(t))

        @pl.loop(0, streams)
        def _(s):
            acc = load(s, tiles[0])
            for rows in tiles[1:]:
                acc += load(s, rows)
            mean_ref[pl.ds(s, 1), :] = jnp.sum(acc, axis=0, keepdims=True)

        mean_ref[...] = group_mean(mean_ref[...])

        @pl.loop(0, streams)
        def _(s):
            keep_reading(s)
            mean = sample_row(mean_ref, s)
            acc = jnp.zeros((SUBLANES, chans), jnp.float32)
            for rows in tiles:
                centered = load(s, rows) - mean
                acc += centered * centered
            scale_ref[pl.ds(s, 1), :] = jnp.sum(acc, axis=0, keepdims=True)

        gamma = g_buf[...].astype(jnp.float32).reshape(1, chans)
        beta = b_buf[...].astype(jnp.float32).reshape(1, chans)
        scale_ref[...] = gamma / jnp.sqrt(group_mean(scale_ref[...]) + EPS)

        @pl.loop(0, streams)
        def _(s):
            keep_reading(streams + s)
            mean, scale = sample_row(mean_ref, s), sample_row(scale_ref, s)
            shift = jnp.broadcast_to(beta, (SUBLANES, chans))
            for rows in tiles:
                y = (load(s, rows) - mean) * scale + shift
                o_buf[s, r, rows, :] = y.astype(o_buf.dtype)

    copy_g = pltpu.make_async_copy(g_hbm, g_buf, sems.at[sem_affine])
    copy_b = pltpu.make_async_copy(b_hbm, b_buf, sems.at[sem_affine])
    copy_g.start(priority=1)
    copy_b.start(priority=1)
    read_steps(0, steps + READ_AHEAD)

    @pl.loop(0, rounds)
    def _(r):
        @pl.when(r < early)
        def _():
            wait_read(r, slice(None), r)

        @pl.when(r == 0)
        def _():
            copy_g.wait()
            copy_b.wait()

        @pl.when(r == early)
        def _():
            read_steps((early + 1) * steps + READ_AHEAD, total)
            wait_read(pl.ds(early, rounds - early - 1), slice(None), sem_late)
            wait_read(rounds - 1, pl.ds(0, head), sem_late)
            write_rounds(0, early)
            wait_read(rounds - 1, pl.ds(head, npos - head), sem_tail)

        normalize_round(r)
        pl.when(r >= early)(lambda: write_rounds(r, r + 1))

    pltpu.make_async_copy(o_buf, o_hbm, sems.at[sem_out]).wait()


@jax.jit
def pallas_standalone__groupnorm__sampling_kernel(
    x: jax.Array,
    g: jax.Array,
    b: jax.Array,
):
    batch, chans, height, width = x.shape
    streams = batch // ROUNDS
    view = (streams, ROUNDS, height * width, chans)
    steps = view[2] // READ_ROWS
    assert batch % (ROUNDS * READ_QUEUES) == 0 and chans % GROUPS == 0
    assert view[2] % WRITE_ROWS == 0 and steps % (2 * streams) == 0
    assert READ_AHEAD % (steps // (2 * streams)) == 0 and OVERLAP < READ_AHEAD <= steps

    in_hbm = pl.BlockSpec(memory_space=pltpu.MemorySpace.HBM)
    out = pl.pallas_call(
        _groupnorm_kernel,
        in_specs=[in_hbm, in_hbm, in_hbm],
        out_specs=in_hbm,
        out_shape=jax.ShapeDtypeStruct(view, x.dtype),
        scratch_shapes=[
            pltpu.VMEM(view, x.dtype),
            pltpu.VMEM(view, x.dtype),
            pltpu.VMEM((chans,), g.dtype),
            pltpu.VMEM((chans,), b.dtype),
            pltpu.VMEM((streams, chans), jnp.float32),
            pltpu.VMEM((streams, chans), jnp.float32),
            pltpu.SemaphoreType.DMA((ROUNDS // 2 + 4,)),
        ],
        compiler_params=pltpu.CompilerParams(
            vmem_limit_bytes=56 * 1024 * 1024,
            disable_bounds_checks=True,
            disable_semaphore_checks=True,
        ),
    )(jnp.transpose(x, (0, 2, 3, 1)).reshape(view), g, b)
    return jnp.transpose(out.reshape(batch, height, width, chans), (0, 3, 1, 2))
```

```python
import jax
import jax.numpy as jnp
from jax import lax
from jax.experimental import pallas as pl
from jax.experimental.pallas import tpu as pltpu

GROUPS = 32
EPS = 1e-5

ROUNDS = 4
READ_QUEUES = 2
READ_ROWS = 8
WRITE_ROWS = 16
READ_AHEAD = 52
OVERLAP = 10

SUBLANES = 8
LANES = 128


def _groupnorm_kernel(
    x_hbm, g_hbm, b_hbm, o_hbm, x_buf, o_buf, g_buf, b_buf, mean_ref, scale_ref, sems
):
    streams, rounds, npos, chans = x_hbm.shape
    group = chans // GROUPS
    early = rounds // 2
    steps = npos // READ_ROWS
    total = rounds * steps
    burst = steps // (2 * streams)
    head = npos - OVERLAP * READ_ROWS
    sem_tail, sem_out, sem_g, sem_b = range(rounds, rounds + 4)

    def read_burst(t):
        r, j = lax.div(t, steps), lax.rem(t, steps)
        width = streams // READ_QUEUES
        for i in range(burst):
            s = jnp.where(t + i < total - OVERLAP, r, sem_tail)
            start = pl.multiple_of((j + i) * READ_ROWS, READ_ROWS)
            for q in range(READ_QUEUES):
                idx = (pl.ds(q * width, width), r, pl.ds(start, READ_ROWS))
                copy = pltpu.make_async_copy(x_hbm.at[idx], x_buf.at[idx], sems.at[s])
                copy.start(priority=q)

    def read_steps(t0, t1):
        pl.loop(t0 // burst, t1 // burst)(lambda u: read_burst(u * burst))

    def wait_read(r, rows, s):
        idx = (slice(None), r, rows)
        pltpu.make_async_copy(x_hbm.at[idx], x_buf.at[idx], sems.at[s]).wait()

    def write_rounds(r0, r1):
        per_round = npos // WRITE_ROWS

        @pl.loop(r0 * per_round, r1 * per_round)
        def _(t):
            start = pl.multiple_of(lax.rem(t, per_round) * WRITE_ROWS, WRITE_ROWS)
            idx = (slice(None), lax.div(t, per_round), pl.ds(start, WRITE_ROWS))
            pltpu.make_async_copy(o_buf.at[idx], o_hbm.at[idx], sems.at[sem_out]).start()

    def group_mean(col_sums):
        width = pl.cdiv(chans, LANES) * LANES
        v = jnp.concatenate(
            [col_sums, jnp.zeros((streams, width - chans), jnp.float32)], axis=1
        )
        lane = lax.broadcasted_iota(jnp.int32, v.shape, 1).astype(jnp.float32)
        pos = lane - group * jnp.floor((lane + 0.5) * (1.0 / group))
        upto = v
        after = jnp.where(pos < group - 1, pltpu.roll(v, width - 1, 1), 0.0)
        d = 1
        while d < group:
            upto += jnp.where(pos >= d, pltpu.roll(upto, d, 1), 0.0)
            after += jnp.where(pos < group - d, pltpu.roll(after, width - d, 1), 0.0)
            d *= 2
        return (upto + after)[:, :chans] * (1.0 / (group * npos))

    def normalize_round(r):
        tiles = [pl.ds(i, SUBLANES) for i in range(0, npos, SUBLANES)]

        def load(s, rows):
            return x_buf[s, r, rows, :].astype(jnp.float32)

        def sample_row(ref, s):
            return jnp.broadcast_to(ref[pl.ds(s, 1), :], (SUBLANES, chans))

        def keep_reading(slot):
            t = (r + 1) * steps + READ_AHEAD + slot * burst
            pl.when(r < early)(lambda: read_burst(t))

        @pl.loop(0, streams)
        def _(s):
            acc = load(s, tiles[0])
            for rows in tiles[1:]:
                acc += load(s, rows)
            mean_ref[pl.ds(s, 1), :] = jnp.sum(acc, axis=0, keepdims=True)

        mean_ref[...] = group_mean(mean_ref[...])

        @pl.loop(0, streams)
        def _(s):
            keep_reading(s)
            mean = sample_row(mean_ref, s)
            acc = jnp.zeros((SUBLANES, chans), jnp.float32)
            for rows in tiles:
                centered = load(s, rows) - mean
                acc += centered * centered
            scale_ref[pl.ds(s, 1), :] = jnp.sum(acc, axis=0, keepdims=True)

        gamma = g_buf[...].astype(jnp.float32).reshape(1, chans)
        beta = b_buf[...].astype(jnp.float32).reshape(1, chans)
        scale_ref[...] = gamma / jnp.sqrt(group_mean(scale_ref[...]) + EPS)

        @pl.loop(0, streams)
        def _(s):
            keep_reading(streams + s)
            mean, scale = sample_row(mean_ref, s), sample_row(scale_ref, s)
            shift = jnp.broadcast_to(beta, (SUBLANES, chans))
            for rows in tiles:
                y = (load(s, rows) - mean) * scale + shift
                o_buf[s, r, rows, :] = y.astype(o_buf.dtype)

    copy_g = pltpu.make_async_copy(g_hbm, g_buf, sems.at[sem_g])
    copy_b = pltpu.make_async_copy(b_hbm, b_buf, sems.at[sem_b])
    copy_g.start(priority=1)
    copy_b.start(priority=1)
    read_steps(0, steps + READ_AHEAD)

    @pl.loop(0, rounds)
    def _(r):
        @pl.when(r < early)
        def _():
            wait_read(r, slice(None), r)

        @pl.when(r == 0)
        def _():
            copy_g.wait()
            copy_b.wait()

        @pl.when(r == early)
        def _():
            read_steps((early + 1) * steps + READ_AHEAD, total)
            for late in range(early, rounds - 1):
                wait_read(late, slice(None), late)
            wait_read(rounds - 1, pl.ds(0, head), rounds - 1)
            write_rounds(0, early)
            wait_read(rounds - 1, pl.ds(head, npos - head), sem_tail)

        normalize_round(r)
        pl.when(r >= early)(lambda: write_rounds(r, r + 1))

    pltpu.make_async_copy(o_buf, o_hbm, sems.at[sem_out]).wait()


@jax.jit
def pallas_standalone__groupnorm__sampling_kernel(
    x: jax.Array,
    g: jax.Array,
    b: jax.Array,
):
    batch, chans, height, width = x.shape
    streams = batch // ROUNDS
    view = (streams, ROUNDS, height * width, chans)
    steps = view[2] // READ_ROWS
    assert batch % (ROUNDS * READ_QUEUES) == 0 and chans % GROUPS == 0
    assert view[2] % WRITE_ROWS == 0 and steps % (2 * streams) == 0
    assert READ_AHEAD % (steps // (2 * streams)) == 0 and OVERLAP < READ_AHEAD <= steps

    in_hbm = pl.BlockSpec(memory_space=pltpu.MemorySpace.HBM)
    out = pl.pallas_call(
        _groupnorm_kernel,
        in_specs=[in_hbm, in_hbm, in_hbm],
        out_specs=in_hbm,
        out_shape=jax.ShapeDtypeStruct(view, x.dtype),
        scratch_shapes=[
            pltpu.VMEM(view, x.dtype),
            pltpu.VMEM(view, x.dtype),
            pltpu.VMEM((chans,), g.dtype),
            pltpu.VMEM((chans,), b.dtype),
            pltpu.VMEM((streams, chans), jnp.float32),
            pltpu.VMEM((streams, chans), jnp.float32),
            pltpu.SemaphoreType.DMA((ROUNDS + 4,)),
        ],
        compiler_params=pltpu.CompilerParams(
            vmem_limit_bytes=56 * 1024 * 1024,
            disable_bounds_checks=True,
            disable_semaphore_checks=True,
        ),
    )(jnp.transpose(x, (0, 2, 3, 1)).reshape(view), g, b)
    return jnp.transpose(out.reshape(batch, height, width, chans), (0, 3, 1, 2))
```
